```python
import os as _os
_os.environ.setdefault("JAX_PLATFORMS", "cpu")
import jax
import jax.numpy as jnp

def _softmax(x, axis=-1):
    return jax.nn.softmax(x, axis=axis)
def _gelu(x):
    return jax.nn.gelu(x, approximate=True)
def _silu(x):
    return jax.nn.silu(x)
def _sigmoid(x):
    return jax.nn.sigmoid(x)
def _layernorm(x, axis=-1, eps=1e-5):
    m = jnp.mean(x, axis=axis, keepdims=True)
    v = jnp.var(x, axis=axis, keepdims=True)
    return (x - m) / jnp.sqrt(v + eps)
def _scatter_add(tgt, idx, src, axis=0):
    return tgt.at[idx].add(src)
def _segment_sum(src, seg, n):
    return jax.ops.segment_sum(src, seg, n)
class _Rng:
    def __init__(self, key):
        self._k = key
    def _next(self):
        self._k, sub = jax.random.split(self._k)
        return sub
    def normal(self, shape):
        return jax.random.normal(self._next(), shape, dtype=jnp.bfloat16)
    def randint(self, lo, hi, shape):
        return jax.random.randint(self._next(), shape, lo, hi, dtype=jnp.int32)
    def uniform(self, shape, lo=0.0, hi=1.0):
        return jax.random.uniform(self._next(), shape, jnp.bfloat16, lo, hi)
    def permutation(self, n):
        return jax.random.permutation(self._next(), n)


kernel_name = 'sequential_preLN__linear_kernel_hedgehog__dense_activation_squared_relu__prompt'

def setup_inputs():
    _rng = _Rng(jax.random.key(int.from_bytes(__import__("os").urandom(4), "little")))
    _w = (lambda a: (lambda t: t.astype(jnp.bfloat16) if jnp.issubdtype(t.dtype, jnp.floating) else t)(jnp.asarray(a)))
    def _A_setup():
        B, S, D, H = 1, 2048, 512, 32
        Dh = D // H
        return {
            "x": _w((lambda *s: _rng.normal(s) * 0.05)(B, S, D)),
            "wqkv": _w((lambda *s: _rng.normal(s) * 0.2)(D, 3 * D)),
            "w_phi": _w((lambda *s: _rng.normal(s) * 0.2)(H, Dh, Dh) * (Dh ** -0.5)),
            "wo": _w((lambda *s: _rng.normal(s) * 0.05)(D, D)),
        }
    _A_in = _A_setup()

    def _B_setup():
        B, S, D, F = 1, 2048, 512, 1792
        return {
            "x": _w((lambda *s: _rng.normal(s) * 0.05)(B, S, D)),
            "w1": _w((lambda *s: _rng.normal(s) * 0.05)(D, F)),
            "b1": _w((lambda *s: _rng.normal(s) * 0.05)(F)),
            "w2": _w((lambda *s: _rng.normal(s) * 0.05)(F, D)),
            "b2": _w((lambda *s: _rng.normal(s) * 0.05)(D)),
        }
    _B_in = _B_setup()

    return {
        "A_x": _A_in["x"],
        "A_wqkv": _A_in["wqkv"],
        "A_w_phi": _A_in["w_phi"],
        "A_wo": _A_in["wo"],
        "B_x": _B_in["x"],
        "B_w1": _B_in["w1"],
        "B_b1": _B_in["b1"],
        "B_w2": _B_in["w2"],
        "B_b2": _B_in["b2"],
    }

def reference(A_x, A_wqkv, A_w_phi, A_wo, B_x, B_w1, B_b1, B_w2, B_b2):
    def _A_ref(x, wqkv, w_phi, wo):
        B, S, D = x.shape
        H = 32; Dh = D // H
        qkv = (lambda x, *d: x.transpose(*d))((x @ wqkv).reshape(B, S, 3, H, Dh), 2, 0, 3, 1, 4)
        q, k, v = qkv[0], qkv[1], qkv[2]
        pq = jnp.einsum("bhsd,hdf->bhsf", q, w_phi)
        pk = jnp.einsum("bhsd,hdf->bhsf", k, w_phi)
        phi_q = jnp.concatenate([_softmax(pq, axis=-1), _softmax(-pq, axis=-1)], axis=-1)
        phi_k = jnp.concatenate([_softmax(pk, axis=-1), _softmax(-pk, axis=-1)], axis=-1)
        kv = jnp.einsum("bhsf,bhsd->bhfd", phi_k, v)
        z  = jnp.einsum("bhsf->bhf", phi_k)
        num = jnp.einsum("bhqf,bhfd->bhqd", phi_q, kv)
        den = jnp.einsum("bhqf,bhf->bhq", phi_q, z)[..., None] + 1e-6
        o = num / den
        return (lambda x, *d: x.transpose(*d))(o, 0, 2, 1, 3).reshape(B, S, D) @ wo

    def _B_ref(x, w1, b1, w2, b2):
        h = jnp.einsum("bsd,df->bsf", x, w1) + b1
        zero = jnp.zeros_like(h)
        r = jnp.where(h > zero, h, zero)
        h = r * r
        out = jnp.einsum("bsf,fd->bsd", h, w2) + b2
        return out

    x = A_x
    h = x + _A_ref(_layernorm(x, axis=-1), A_wqkv, A_w_phi, A_wo)
    h2 = h + _B_ref(_layernorm(h, axis=-1), B_w1, B_b1, B_w2, B_b2)
    return h2
```

```python
import functools
import math
import jax
import jax.numpy as jnp
from jax import lax
from jax.experimental import pallas as pl
from jax.experimental.pallas import tpu as pltpu

NT = (((1,), (1,)), ((), ()))
NN = (((1,), (0,)), ((), ()))
TN = (((0,), (0,)), ((), ()))
F32 = jnp.float32
BF16 = jnp.bfloat16
LOG2E = math.log2(math.e)


def _dot(a, b, dn=NN):
    return lax.dot_general(a, b, dn, preferred_element_type=F32)


def _ln(x):
    m = jnp.mean(x, axis=-1, keepdims=True)
    c = x - m
    v = jnp.mean(c * c, axis=-1, keepdims=True)
    return c * lax.rsqrt(v + 1e-5)


def _allred(op, a):
    r = a[0]
    for i in range(1, a.shape[0]):
        r = op(r, a[i])
    return op(r, pltpu.roll(r, 4, 0))[None]


def _rcp(s):
    r = pl.reciprocal(s, approx=True)
    return r * (2.0 - s * r)


def _phi(p, RCP=0):
    t = p.shape[1]
    p3 = p.reshape(8, 8, t)
    mx = _allred(jnp.maximum, p3)
    mn = _allred(jnp.minimum, p3)
    e1 = jnp.exp2(p3 - mx)
    e2 = jnp.exp2(mn - p3)
    if RCP:
        r1 = _rcp(_allred(jnp.add, e1))
        r2 = _rcp(_allred(jnp.add, e2))
    else:
        r1 = 1.0 / _allred(jnp.add, e1)
        r2 = 1.0 / _allred(jnp.add, e2)
    a = (e1 * r1).reshape(64, t)
    b = (e2 * r2).reshape(64, t)
    return jnp.concatenate([a, b], axis=0)


def make_kernel(T1, T2, SUB, RC, FORD, FSUB, P0, LNP, LQ, UN1, RCP, DV):
    S, D, F = 2048, 512, 1792
    n1, n2 = S // T1, S // T2
    nsub = T2 // FSUB
    XC = 256

    def kernel(x_hbm, wqkv_hbm, wphi_hbm, wo_hbm, w1_hbm, b1_hbm, w2_hbm, b2_hbm, out_hbm,
               x_v, xn_v, wqkv_v, wt_v, wo_v, w1_v, w2_v, kv_acc, z_acc, kv_bf, out_v, wphi_v, b1_v, b2_v,
               sems, xsem, osem):
        cp_wk = pltpu.make_async_copy(wqkv_hbm.at[:, D:2 * D], wqkv_v.at[:, D:2 * D], sems.at[0])
        cp_wv = pltpu.make_async_copy(wqkv_hbm.at[:, 2 * D:], wqkv_v.at[:, 2 * D:], sems.at[1])
        cp_wq = pltpu.make_async_copy(wqkv_hbm.at[:, :D], wqkv_v.at[:, :D], sems.at[2])
        cp_wo = pltpu.make_async_copy(wo_hbm, wo_v, sems.at[3])
        cp_w1 = pltpu.make_async_copy(w1_hbm, w1_v, sems.at[4])
        cp_w2 = pltpu.make_async_copy(w2_hbm, w2_v, sems.at[5])
        cp_wp = pltpu.make_async_copy(wphi_hbm, wphi_v, sems.at[6])
        cp_b1 = pltpu.make_async_copy(b1_hbm, b1_v, sems.at[7])
        cp_b2 = pltpu.make_async_copy(b2_hbm, b2_v, sems.at[8])

        def rows_of(i, T):
            return pl.ds(i * T if isinstance(i, int) else pl.multiple_of(i * T, T), T)

        def cp_x(i, T):
            rows = rows_of(i, T)
            return pltpu.make_async_copy(x_hbm.at[rows], x_v.at[rows], xsem.at[i * (T // XC)])

        cp_wp.start()
        cp_x(0, XC).start()

        rr = lax.broadcasted_iota(jnp.int32, (512, 32), 0)
        cc = lax.broadcasted_iota(jnp.int32, (512, 32), 1)
        hsel = (cc == (rr // 64) * 4 + rr % 4).astype(F32).astype(BF16)
        r2 = lax.broadcasted_iota(jnp.int32, (512, 256), 0)
        c2 = lax.broadcasted_iota(jnp.int32, (512, 256), 1)
        fmask = (c2 % 16) == (r2 % 64) // 4
        r3 = lax.broadcasted_iota(jnp.int32, (256, 128), 0)
        c3 = lax.broadcasted_iota(jnp.int32, (256, 128), 1)
        dsel = (r3 // 16 == c3 % 16).astype(F32).astype(BF16)
        r4 = lax.broadcasted_iota(jnp.int32, (512, 128), 0)
        c4 = lax.broadcasted_iota(jnp.int32, (512, 128), 1)
        hmask = (c4 // 16) == ((r4 % 128) // 64) * 4 + r4 % 4
        cp_wp.wait()
        cp_wk.start()
        t = _dot(hsel, wphi_v[...], NT)
        t = jnp.where(fmask, t, 0.0).astype(BF16)
        t = _dot(t, dsel)
        bdt = jnp.where(hmask, t, 0.0).astype(BF16)
        kv_acc[...] = jnp.zeros(kv_acc.shape, F32)
        z_acc[...] = jnp.zeros(z_acc.shape, F32)

        def ln_rows(rows):
            xn_v[rows, :] = _ln(x_v[rows, :].astype(F32)).astype(BF16)

        cp_x(0, XC).wait()
        cp_x(1, XC).start()
        ln_rows(rows_of(0, XC))
        cp_wk.wait()
        cp_wv.start()
        for g in range(4):
            wk = wqkv_v[:, D + g * 128:D + (g + 1) * 128]
            wt_v[D + g * 128:D + (g + 1) * 128, :] = (_dot(bdt[g * 128:(g + 1) * 128], wk, NT) * LOG2E).astype(BF16)

        def kv_update(j, pk, vg):
            phi = _phi(pk, RCP)
            zs = phi[:, :128]
            for c0 in range(128, phi.shape[1], 128):
                zs = zs + phi[:, c0:c0 + 128]
            z_acc[j] += zs
            kv_acc[j] += _dot(vg.astype(BF16), phi.astype(BF16), NT)

        cp_x(1, XC).wait()
        cp_x(1, T1).start()
        pk0a = _dot(wt_v[D:2 * D, :], xn_v[rows_of(0, XC), :], NT)
        ln_rows(rows_of(1, XC))
        cp_wv.wait()
        for i in range(2, n1):
            cp_x(i, T1).start()
        pk0b = _dot(wt_v[D:2 * D, :], xn_v[rows_of(1, XC), :], NT)
        wt_v[2 * D:, :] = wqkv_v[:, 2 * D:].T
        def phi_z(j, pk):
            phi = _phi(pk[j * 64:(j + 1) * 64], RCP)
            zs = phi[:, :128]
            for c0 in range(128, phi.shape[1], 128):
                zs = zs + phi[:, c0:c0 + 128]
            z_acc[j] += zs
            return phi.astype(BF16)
        pha = [phi_z(j, pk0a) for j in range(8)]
        cp_x(1, T1).wait()
        cp_wq.start()
        cp_wo.start()
        cp_w1.start()
        cp_w2.start()
        cp_b1.start()
        cp_b2.start()
        for j0 in range(0, 8, P0):
            vt0 = _dot(wt_v[2 * D + j0 * 64:2 * D + (j0 + P0) * 64, :], xn_v[rows_of(0, T1), :], NT)
            for j in range(j0, j0 + P0):
                if j == LQ:
                    ln_rows(rows_of(1, T1))
                phi = jnp.concatenate([pha[j], phi_z(j, pk0b)], axis=1)
                kv_acc[j] += _dot(vt0[(j - j0) * 64:(j - j0 + 1) * 64].astype(BF16), phi, NT)

        def body1(i, carry):
            @pl.when(i < n1 - 1)
            def _():
                cp_x(jnp.minimum(i + 1, n1 - 1), T1).wait()
            kvt = _dot(wt_v[D:, :], xn_v[rows_of(i, T1), :], NT)
            for j in range(8):
                if j == LNP:
                    ln_rows(rows_of(jnp.minimum(i + 1, n1 - 1), T1))
                kv_update(j, kvt[j * 64:(j + 1) * 64], kvt[D + j * 64:D + (j + 1) * 64])
            return carry
        if UN1:
            for i in range(2, n1):
                cp_x(i, T1).wait()
            cp_wq.wait()
            for i in range(1, n1):
                if i + 1 < n1 and UN1 == 1:
                    ln_rows(rows_of(i + 1, T1))
                kvt = _dot(wt_v[D:, :], xn_v[rows_of(i, T1), :], NT)
                if i + 1 < n1 and UN1 == 2:
                    ln_rows(rows_of(i + 1, T1))
                for j in range(8):
                    kv_update(j, kvt[j * 64:(j + 1) * 64], kvt[D + j * 64:D + (j + 1) * 64])
        else:
            lax.fori_loop(1, n1, body1, 0)

        for g in range(4):
            wq = wqkv_v[:, g * 128:(g + 1) * 128]
            wt_v[g * 128:(g + 1) * 128, :] = (_dot(bdt[g * 128:(g + 1) * 128], wq, NT) * LOG2E).astype(BF16)
        r5 = lax.broadcasted_iota(jnp.int32, (64, 128), 0)
        c5 = lax.broadcasted_iota(jnp.int32, (64, 128), 1)
        kmask = (r5 // 16) == (c5 % 4)
        r6 = lax.broadcasted_iota(jnp.int32, (16, 128), 0)
        c6 = lax.broadcasted_iota(jnp.int32, (16, 128), 1)
        zmask = r6 == (c6 % 4)
        ones = jnp.ones((16, 128), BF16)
        for j in range(8):
            kv_bf[j, :64, :] = jnp.where(kmask, kv_acc[j], 0.0).astype(BF16)
            if DV:
                z_acc[j] = jnp.broadcast_to(jnp.sum(z_acc[j], axis=1, keepdims=True), (128, 128))
            else:
                zt = _dot(ones, z_acc[j].astype(BF16), NT)
                kv_bf[j, 64:, :] = jnp.where(zmask, zt, 0.0).astype(BF16)
        cp_wo.wait()
        cp_w1.wait()
        cp_w2.wait()
        cp_b1.wait()
        cp_b2.wait()
        b1 = b1_v[...].astype(F32).reshape(1, F)
        b2 = b2_v[...].astype(F32).reshape(1, D)

        def cp_out(i):
            rows = rows_of(i, FSUB)
            return pltpu.make_async_copy(out_v.at[rows], out_hbm.at[rows], osem.at[i])

        def p2(i, carry):
            base = pl.multiple_of(i * T2, T2)
            ots = []
            for s0 in range(0, T2, SUB):
                qt = _dot(wt_v[:D, :], xn_v[pl.ds(base + s0, SUB), :], NT)
                og = []
                for j in range(8):
                    phi = _phi(qt[j * 64:(j + 1) * 64], RCP)
                    if DV:
                        nd = _dot(kv_bf[j, :64, :], phi.astype(BF16))
                        zr = z_acc[j]
                        zr = jnp.concatenate([zr] * (SUB // 128), axis=1)
                        den = _allred(jnp.add, (phi * zr).reshape(16, 8, SUB))[0]
                    else:
                        nd = _dot(kv_bf[j], phi.astype(BF16))
                        den = nd[64:72]
                    rden = _rcp(den + 1e-6) if RCP else 1.0 / (den + 1e-6)
                    for h in range(4):
                        o = nd[h * 16:(h + 1) * 16] * rden[h:h + 1]
                        og.append(o.astype(BF16))
                ots.append(jnp.concatenate(og, axis=0))
            ot = jnp.concatenate(ots, axis=1)
            hs, hns = [], []
            for r0 in range(0, T2, RC):
                xr = x_v[pl.ds(base + r0, RC), :]
                h = xr.astype(F32) + _dot(ot[:, r0:r0 + RC], wo_v[...], TN)
                hs.append(h + b2)
                hns.append(_ln(h).astype(BF16))
            hn = jnp.concatenate(hns, axis=0)
            acc = jnp.concatenate(hs, axis=0)

            def f1(s):
                hid = _dot(hn[s * FSUB:(s + 1) * FSUB], w1_v[...]) + b1
                hid = jnp.maximum(hid, 0.0)
                return (hid * hid).astype(BF16)

            def f2(s, hid):
                o = acc[s * FSUB:(s + 1) * FSUB] + _dot(hid, w2_v[...])
                out_v[pl.ds(base + s * FSUB, FSUB), :] = o.astype(BF16)
                cp_out(i * nsub + s).start()

            if FORD == 0:
                hids = [f1(s) for s in range(nsub)]
                for s in range(nsub):
                    f2(s, hids[s])
            else:
                for s in range(nsub):
                    f2(s, f1(s))
            return carry

        lax.fori_loop(0, n2, p2, 0)
        for i in range(n2 * nsub):
            cp_out(i).wait()

    hbm = pl.BlockSpec(memory_space=pltpu.HBM)
    call = pl.pallas_call(
        kernel,
        out_shape=jax.ShapeDtypeStruct((S, D), BF16),
        in_specs=[hbm] * 8,
        out_specs=hbm,
        scratch_shapes=[
            pltpu.VMEM((S, D), BF16), pltpu.VMEM((S, D), BF16),
            pltpu.VMEM((D, 3 * D), BF16), pltpu.VMEM((3 * D, D), BF16),
            pltpu.VMEM((D, D), BF16),
            pltpu.VMEM((D, F), BF16), pltpu.VMEM((F, D), BF16),
            pltpu.VMEM((8, 64, 128), F32), pltpu.VMEM((8, 128, 128), F32), pltpu.VMEM((8, 80, 128), BF16),
            pltpu.VMEM((S, D), BF16),
            pltpu.VMEM((256, 32), BF16), pltpu.VMEM((F,), BF16), pltpu.VMEM((D,), BF16),
            pltpu.SemaphoreType.DMA((9,)), pltpu.SemaphoreType.DMA((S // XC,)), pltpu.SemaphoreType.DMA((n2 * nsub,)),
        ],
        compiler_params=pltpu.CompilerParams(vmem_limit_bytes=96 * 1024 * 1024),
        name="fused_block",
    )

    def fn(A_x, A_wqkv, A_w_phi, A_wo, B_x, B_w1, B_b1, B_w2, B_b2):
        wp = A_w_phi.transpose(1, 2, 0).reshape(256, 32)
        out = call(A_x.reshape(S, D), A_wqkv, wp, A_wo, B_w1, B_b1, B_w2, B_b2)
        return out.reshape(1, S, D)
    return fn


_impl = make_kernel(T1=512, T2=1024, SUB=256, RC=128, FORD=1, FSUB=256, P0=2, LNP=0, LQ=0, UN1=2, RCP=1, DV=1)


@jax.jit
def pallas_sequential_preLN__linear_kernel_hedgehog__dense_activation_squared_relu__prompt_kernel(
    A_x, A_wqkv, A_w_phi, A_wo, B_x, B_w1, B_b1, B_w2, B_b2):
    return _impl(A_x, A_wqkv, A_w_phi, A_wo, B_x, B_w1, B_b1, B_w2, B_b2)
```

```python
import math

import jax
import jax.numpy as jnp
from jax import lax
from jax.experimental import pallas as pl
from jax.experimental.pallas import tpu as pltpu

F32 = jnp.float32
BF16 = jnp.bfloat16
U32 = jnp.uint32
NN = (((1,), (0,)), ((), ()))
NT = (((1,), (1,)), ((), ()))
TN = (((0,), (0,)), ((), ()))
LOG2E = math.log2(math.e)


def _dot(a, b, dims=NN):
    return lax.dot_general(a, b, dims, preferred_element_type=F32)


def _iota(shape, axis):
    return lax.broadcasted_iota(jnp.int32, shape, axis)


def _layernorm(x):
    c = x - jnp.mean(x, axis=-1, keepdims=True)
    v = jnp.mean(c * c, axis=-1, keepdims=True)
    return c * lax.rsqrt(v + 1e-5)


def _recip(s):
    r = pl.reciprocal(s, approx=True)
    return r * (2.0 - s * r)


def _head_reduce(op, a):
    r = a[0]
    for i in range(1, a.shape[0]):
        r = op(r, a[i])
    return op(r, pltpu.roll(r, 4, 0))


def _hedgehog(p):
    t = p.shape[1]
    p = p.reshape(8, 8, t)
    e_pos = jnp.exp2(p - _head_reduce(jnp.maximum, p)[None])
    e_neg = jnp.exp2(_head_reduce(jnp.minimum, p)[None] - p)
    pos = e_pos * _recip(_head_reduce(jnp.add, e_pos))[None]
    neg = e_neg * _recip(_head_reduce(jnp.add, e_neg))[None]
    return jnp.concatenate([pos, neg], axis=0)


S, D, F = 2048, 512, 1792
T1 = 512
T2 = 1024
SUB = 128
C0 = XC = 256
P0, JD = 4, 5
QA, WD, FD = 1, 1, 2


def _make_call():
    n1, n2, ns = S // T1, S // T2, T2 // SUB
    cuts = [0, C0] + list(range(C0 + XC, T1 + 1, XC))
    x_pieces = list(zip(cuts[:-1], cuts[1:])) + [(i * T1, (i + 1) * T1) for i in range(1, n1)]
    nx0 = len(cuts) - 1
    assert cuts[-1] == T1

    def kernel(x_hbm, wqkv_hbm, wphi_hbm, wo_hbm, w1_hbm, b1_hbm, w2_hbm, b2_hbm, out_hbm,
               x_v, xn_v, wqkv_v, wt_v, wo_v, w1_v, w2_v, kv_v, z_v, kvm_v, out_v, wphi_v, b1_v, b2_v,
               isem, osem):
        def load(ref, r0, n):
            start = r0 // 2 if isinstance(r0, int) else pl.multiple_of(r0 // 2, n // 2)
            return pltpu.bitcast(ref[pl.ds(start, n // 2), :], BF16)

        def store(ref, r0, val):
            ref[pl.ds(r0 // 2, val.shape[0] // 2), :] = pltpu.bitcast(val.astype(BF16), U32)

        def cols(ref, c0, n):
            return ref.at[:, c0:c0 + n]

        copies = {
            "wphi": (wphi_hbm, wphi_v),
            "wk0": (cols(wqkv_hbm, D, D // 2), cols(wqkv_v, D, D // 2)),
            "wk1": (cols(wqkv_hbm, D + D // 2, D // 2), cols(wqkv_v, D + D // 2, D // 2)),
            "wv": (cols(wqkv_hbm, 2 * D, D), cols(wqkv_v, 2 * D, D)),
            "wq": (cols(wqkv_hbm, 0, D), cols(wqkv_v, 0, D)),
            "wo": (wo_hbm, wo_v), "w1": (w1_hbm, w1_v), "w2": (w2_hbm, w2_v),
            "b1": (b1_hbm, b1_v), "b2": (b2_hbm, b2_v),
        }
        for i, (a, b) in enumerate(x_pieces):
            copies["x%d" % i] = (x_hbm.at[a:b], x_v.at[a:b])
        names = list(copies)

        def copy(name, zero=0):
            src, dst = copies[name]
            return pltpu.make_async_copy(src, dst, isem.at[names.index(name) + zero])

        def wait(name, after=None):
            zero = 0 if after is None else (after[-1, -1] > jnp.inf).astype(jnp.int32)
            copy(name, zero).wait()
            return zero

        order = (["wphi", "x0", "wk0", "wk1"] + ["x%d" % i for i in range(1, nx0)] + ["wv"]
                 + ["x%d" % i for i in range(nx0, len(x_pieces))] + ["wq", "wo", "w1", "w2", "b1", "b2"])
        for name in order:
            copy(name).start()

        r, c = _iota((128, 256), 0), _iota((128, 256), 1)
        f_mask = (c % 16) == (r % 64) // 4
        r, c = _iota((128, 128), 0), _iota((128, 128), 1)
        h_mask = (c // 16) == (r // 64) * 4 + r % 4
        r, c = _iota((256, 128), 0), _iota((256, 128), 1)
        d_sel = (r // 16 == c % 16).astype(F32).astype(BF16)
        r, c = _iota((512, 32), 0), _iota((512, 32), 1)
        h_sel = (c == (r // 64) * 4 + r % 4).astype(F32).astype(BF16)

        def block_diag(g0, g1):
            t0 = _dot(h_sel[g0 * 128:g1 * 128], wphi_v[...], NT)
            t = jnp.concatenate([jnp.where(f_mask, t0[i * 128:(i + 1) * 128], 0.0) for i in range(g1 - g0)], axis=0)
            t = _dot(t.astype(BF16), d_sel)
            return t0, t, [jnp.where(h_mask, t[i * 128:(i + 1) * 128], 0.0).astype(BF16) for i in range(g1 - g0)]

        def fold(bd, c0):
            w = _dot(bd, wqkv_v[:, c0:c0 + 128], NT) * LOG2E
            store(wt_v, c0, w)
            return w

        def norm_x(r0, n):
            store(xn_v, r0, _layernorm(x_v[r0:r0 + n, :].astype(F32)))

        def k_features(j, pk):
            phi = _hedgehog(pk[j * 64:(j + 1) * 64])
            t = phi.shape[2]
            zs = phi[:, :, :128]
            for c0 in range(128, t, 128):
                zs = zs + phi[:, :, c0:c0 + 128]
            z_v[j] += zs
            return phi.reshape(128, t).astype(BF16)

        def kv_update(j, phi, vt):
            kv = _dot(vt.astype(BF16), phi, NT)
            kv_v[j] += kv
            return kv

        wait("wphi")
        t0, t, bd = block_diag(0, 2)
        kv_v[...] = jnp.zeros(kv_v.shape, F32)
        z_v[...] = jnp.zeros(z_v.shape, F32)
        wait("x0", t0[:8])
        norm_x(0, C0)
        bd += block_diag(2, 4)[2]
        xn0 = load(xn_v, 0, C0)
        pk, dep = [], t
        for half in range(2):
            wait("wk%d" % half, dep)
            for g in (2 * half, 2 * half + 1):
                w = fold(bd[g], D + g * 128)
            if half == 1:
                wait("x1", w)
            pk.append(_dot(load(wt_v, D + half * 256, 256), xn0, NT))
            dep = pk[-1][:8, :128]
        pk = [jnp.concatenate(pk, axis=0)]
        phis = []
        for i in range(1, nx0):
            a, b = x_pieces[i]
            if i > 1:
                wait("x%d" % i, pk[-1][:8, :128])
            norm_x(a, b - a)
            if i == 1:
                wait("wv", pk[0][:, :128])
            pk.append(_dot(load(wt_v, D, D), load(xn_v, a, b - a), NT))
            if i == 1:
                store(wt_v, 2 * D, wqkv_v[:, 2 * D:].T)
            phis.append([k_features(j, pk[i - 1]) for j in range(8)])
        wait("x%d" % nx0, pk[-1][:, :128])
        for j0 in range(0, 8, P0):
            vt = _dot(load(wt_v, 2 * D + j0 * 64, P0 * 64), load(xn_v, 0, T1), NT)
            for j in range(j0, j0 + P0):
                if j == 0:
                    norm_x(T1, T1)
                phi = jnp.concatenate([p[j] for p in phis] + [k_features(j, pk[-1])], axis=1)
                kv = kv_update(j, phi, vt[(j - j0) * 64:(j - j0 + 1) * 64])
                if j == JD:
                    dep = kv
        zero = wait("x%d" % (nx0 + 1), dep)
        for i in range(nx0 + 2, len(x_pieces)):
            wait("x%d" % i)
        wait("wq")

        @pl.when(zero == 0)
        def _():
            for i in range(1, n1):
                kvt = _dot(load(wt_v, D, 2 * D), load(xn_v, i * T1, T1), NT)
                if i + 1 < n1:
                    norm_x((i + 1) * T1, T1)
                for j in range(8):
                    kv_update(j, k_features(j, kvt), kvt[D + j * 64:D + (j + 1) * 64])
            for g in range(4):
                fold(bd[g], g * 128)
            r, c = _iota((64, 128), 0), _iota((64, 128), 1)
            same_head = (r // 16) == (c % 4)
            for j in range(8):
                kvm_v[j] = jnp.where(same_head, kv_v[j], 0.0).astype(BF16)
                z_v[j] = jnp.broadcast_to(jnp.sum(z_v[j], axis=2, keepdims=True), z_v.shape[1:])

        wait("wo", z_v[7, 15])
        for name in ("w1", "w2", "b1", "b2"):
            wait(name)
        b1 = b1_v[...].astype(F32).reshape(1, F)
        b2 = b2_v[...].astype(F32).reshape(1, D)

        def out_copy(i):
            rows = pl.ds(i * SUB if isinstance(i, int) else pl.multiple_of(i * SUB, SUB), SUB)
            return pltpu.make_async_copy(out_v.at[rows], out_hbm.at[rows], osem.at[i])

        def query_tile(i, carry):
            base = pl.multiple_of(i * T2, T2)
            pq, ot, res, hn = {}, {}, {}, {}

            def project(s):
                pq[s] = _dot(load(wt_v, 0, D), load(xn_v, base + s * SUB, SUB), NT)

            def attend(s):
                o = []
                for j in range(8):
                    phi = _hedgehog(pq[s][j * 64:(j + 1) * 64])
                    num = _dot(kvm_v[j], phi.reshape(128, SUB).astype(BF16))
                    z = jnp.concatenate([z_v[j]] * (SUB // 128), axis=2)
                    rden = _recip(_head_reduce(jnp.add, phi * z) + 1e-6)
                    for h in range(4):
                        o.append((num[h * 16:(h + 1) * 16] * rden[h:h + 1]).astype(BF16))
                ot[s] = jnp.concatenate(o, axis=0)

            def mix(s):
                a, b = [], []
                for r0 in range(0, SUB, 128):
                    x = x_v[pl.ds(base + s * SUB + r0, 128), :].astype(F32)
                    h = x + _dot(ot[s][:, r0:r0 + 128], wo_v[...], TN)
                    a.append(h + b2)
                    b.append(_layernorm(h).astype(BF16))
                res[s] = jnp.concatenate(a, axis=0)
                hn[s] = jnp.concatenate(b, axis=0)

            def ffn(s):
                a = jnp.maximum(_dot(hn[s], w1_v[...]) + b1, 0.0)
                y = res[s] + _dot((a * a).astype(BF16), w2_v[...])
                out_v[pl.ds(base + s * SUB, SUB), :] = y.astype(BF16)
                out_copy(i * ns + s).start()

            for step in range(-QA, ns + FD):
                for stage, lag in ((project, -QA), (attend, 0), (mix, WD), (ffn, FD)):
                    if 0 <= step - lag < ns:
                        stage(step - lag)
            return carry

        lax.fori_loop(0, n2, query_tile, 0)
        for i in range(n2 * ns):
            out_copy(i).wait()

    hbm = pl.BlockSpec(memory_space=pltpu.HBM)
    call = pl.pallas_call(
        kernel,
        out_shape=jax.ShapeDtypeStruct((S, D), BF16),
        in_specs=[hbm] * 8,
        out_specs=hbm,
        scratch_shapes=[
            pltpu.VMEM((S, D), BF16), pltpu.VMEM((S // 2, D), U32),
            pltpu.VMEM((D, 3 * D), BF16), pltpu.VMEM((3 * D // 2, D), U32),
            pltpu.VMEM((D, D), BF16), pltpu.VMEM((D, F), BF16), pltpu.VMEM((F, D), BF16),
            pltpu.VMEM((8, 64, 128), F32), pltpu.VMEM((8, 16, 8, 128), F32), pltpu.VMEM((8, 64, 128), BF16),
            pltpu.VMEM((S, D), BF16),
            pltpu.VMEM((256, 32), BF16), pltpu.VMEM((F,), BF16), pltpu.VMEM((D,), BF16),
            pltpu.SemaphoreType.DMA((10 + len(x_pieces),)), pltpu.SemaphoreType.DMA((n2 * ns,)),
        ],
        compiler_params=pltpu.CompilerParams(
            vmem_limit_bytes=96 * 1024 * 1024, flags={"XLA_TPU_RESCHEDULE_DMA_DONES": True}),
        name="fused_block",
    )

    return call


@jax.jit
def pallas_sequential_preLN__linear_kernel_hedgehog__dense_activation_squared_relu__prompt_kernel(
    A_x: jax.Array,
    A_wqkv: jax.Array,
    A_w_phi: jax.Array,
    A_wo: jax.Array,
    B_x: jax.Array,
    B_w1: jax.Array,
    B_b1: jax.Array,
    B_w2: jax.Array,
    B_b2: jax.Array,
):
    del B_x
    w_phi = A_w_phi.transpose(1, 2, 0).reshape(256, 32)
    out = _make_call()(A_x.reshape(S, D), A_wqkv, w_phi, A_wo, B_w1, B_b1, B_w2, B_b2)
    return out.reshape(1, S, D)
```
